```python
import os as _os
_os.environ.setdefault("JAX_PLATFORMS", "cpu")
import jax
import jax.numpy as jnp

def _softmax(x, axis=-1):
    return jax.nn.softmax(x, axis=axis)
def _gelu(x):
    return jax.nn.gelu(x, approximate=True)
def _silu(x):
    return jax.nn.silu(x)
def _sigmoid(x):
    return jax.nn.sigmoid(x)
def _layernorm(x, axis=-1, eps=1e-5):
    m = jnp.mean(x, axis=axis, keepdims=True)
    v = jnp.var(x, axis=axis, keepdims=True)
    return (x - m) / jnp.sqrt(v + eps)
def _scatter_add(tgt, idx, src, axis=0):
    return tgt.at[idx].add(src)
def _segment_sum(src, seg, n):
    return jax.ops.segment_sum(src, seg, n)
class _Rng:
    def __init__(self, key):
        self._k = key
    def _next(self):
        self._k, sub = jax.random.split(self._k)
        return sub
    def normal(self, shape):
        return jax.random.normal(self._next(), shape, dtype=jnp.bfloat16)
    def randint(self, lo, hi, shape):
        return jax.random.randint(self._next(), shape, lo, hi, dtype=jnp.int32)
    def uniform(self, shape, lo=0.0, hi=1.0):
        return jax.random.uniform(self._next(), shape, jnp.bfloat16, lo, hi)
    def permutation(self, n):
        return jax.random.permutation(self._next(), n)


kernel_name = 'concat_heads__ssm_conv_h3__sliding_block__prompt'

def setup_inputs():
    _rng = _Rng(jax.random.key(int.from_bytes(__import__("os").urandom(4), "little")))
    _w = (lambda a: (lambda t: t.astype(jnp.bfloat16) if jnp.issubdtype(t.dtype, jnp.floating) else t)(jnp.asarray(a)))
    def _A_setup():
        B, S, D = 1, 2048, 512
        ks = 4
        return {
            "q": _w((lambda *s: _rng.normal(s) * 0.05)(B, S, D)),
            "k": _w((lambda *s: _rng.normal(s) * 0.2)(B, S, D)),
            "v": _w((lambda *s: _rng.normal(s) * 0.2)(B, S, D)),
            "shift_k": _w((lambda *s: _rng.normal(s) * 0.2)(D, ks) * 0.5),
            "ssm_k": _w((lambda *s: _rng.normal(s) * 0.2)(D, S) * (1.0 / S ** 0.5)),
            "ssm_D": _w((lambda *s: _rng.normal(s) * 0.2)(D)),
        }
    _A_in = _A_setup()

    def _B_setup():
        B, S, D = 1, 2048, 512
        return {
            "x": _w((lambda *s: _rng.normal(s) * 0.2)(B, S, D)),
            "wqkv": _w((lambda *s: _rng.normal(s) * 0.2)(D, 3 * D)),
            "wo": _w((lambda *s: _rng.normal(s) * 0.05)(D, D)),
        }
    _B_in = _B_setup()

    return {
        "A_q": _A_in["q"],
        "A_k": _A_in["k"],
        "A_v": _A_in["v"],
        "A_shift_k": _A_in["shift_k"],
        "A_ssm_k": _A_in["ssm_k"],
        "A_ssm_D": _A_in["ssm_D"],
        "B_x": _B_in["x"],
        "B_wqkv": _B_in["wqkv"],
        "B_wo": _B_in["wo"],
    }

def reference(A_q, A_k, A_v, A_shift_k, A_ssm_k, A_ssm_D, B_x, B_wqkv, B_wo):
    def _A_ref(q, k, v, shift_k, ssm_k, ssm_D):
        B, S, D = q.shape
        ks = shift_k.shape[-1]
        k_pad = jnp.pad(k, ((0, 0), (ks - 1, 0), (0, 0)))
        k_shift = jnp.zeros_like(k)
        for t in range(ks):
            k_shift = k_shift + k_pad[:, t:t + S, :] * shift_k[:, ks - 1 - t][None, None, :]
        kv = k_shift * v
        L = 2 * S
        kv_pad = jnp.pad(kv, ((0, 0), (0, S), (0, 0)))
        kf_pad = jnp.pad(ssm_k, ((0, 0), (0, S)))
        kv_f = (lambda x, axes=(-2,-1): jnp.fft.rfft2(x.astype(jnp.float32), axes=axes))(kv_pad[:, None, :, :], axes=(1, 2))
        kf_f = (lambda x, axes=(-2,-1): jnp.fft.rfft2(x.astype(jnp.float32), axes=axes))(kf_pad[:, None, :], axes=(1, 2))
        kf_f = (lambda x, *d: x.transpose(*d))(kf_f, 1, 2, 0)
        y_f = kv_f * kf_f[None, :, :, :]
        y = (lambda x, s, axes=(-2,-1): jnp.fft.irfft2(x, s=s, axes=axes).astype(jnp.bfloat16))(y_f, (1, L), axes=(1, 2))[:, 0, :S, :]
        y = y + kv * ssm_D[None, None, :]
        return q * y

    def _B_ref(x, wqkv, wo):
        B, S, D = x.shape
        H = 32; Dh = D // H; W = 256
        qkv = (lambda x, *d: x.transpose(*d))((x @ wqkv).reshape(B, S, 3, H, Dh), 2, 0, 3, 1, 4)
        q, k, v = qkv[0], qkv[1], qkv[2]
        scores = jnp.einsum("bhqd,bhkd->bhqk", q, k) * (Dh ** -0.5)
        idx = jnp.arange(S)
        mask = (idx[:, None] - idx[None, :] >= 0) & (idx[:, None] - idx[None, :] < W)
        scores = jnp.where(mask[None, None], scores, -1e9)
        p = _softmax(scores, axis=-1)
        o = jnp.einsum("bhqk,bhkd->bhqd", p, v)
        return (lambda x, *d: x.transpose(*d))(o, 0, 2, 1, 3).reshape(B, S, D) @ wo

    a = _A_ref(A_q, A_k, A_v, A_shift_k, A_ssm_k, A_ssm_D)
    b = _B_ref(B_x, B_wqkv, B_wo)
    return jnp.concatenate([a, b], axis=-1)
```

```python
import math
import numpy as np
import ml_dtypes
import jax
import jax.numpy as jnp
from jax import lax
import jax.experimental.pallas as pl
import jax.experimental.pallas.tpu as pltpu

S, D, C, NC = 2048, 512, 128, 16
W = 256
BF = jnp.bfloat16
F32 = jnp.float32

def _dft_consts():
    f = np.arange(128)[:, None].astype(np.float64)
    fw, inv = [], []
    for m in range(4):
        t = (np.arange(128)[None, :] + 128 * m).astype(np.float64)
        ang = np.pi * (2 * f + 1) * t / 256.0
        fw.append(np.concatenate([np.cos(ang), -np.sin(ang)], 0))
        inv.append(np.concatenate([np.cos(ang).T, -np.sin(ang).T], 1) / 128.0)
    return (np.stack(fw).astype(ml_dtypes.bfloat16), np.stack(inv).astype(ml_dtypes.bfloat16))
_FW, _INV = _dft_consts()
NT = (((1,), (1,)), ((), ()))


I32 = jnp.int32
GQ = True
def pk(x): return pltpu.bitcast(x, I32)
def up(x): return pltpu.bitcast(x, BF)

def kern(q_h, k_h, v_h, sk_ref, h_h, sd_ref, x_h, wqkv_h, wo_h, fw_ref, inv_ref, o_h,
         q_ref, k_ref, v_ref, h_ref, x_ref, wqkv_ref, wo_ref, o_ref, sem, osem,
         wT_s, wk_s, wo_s, qT_s, k_s, vT_s, oT_s, bias_s, sc_s, mk_s, kf_s, kv_s, U_s, H_s, Y_s):
    qscale = 0.25 * math.log2(math.e)
    H2 = S // 2
    mk = pltpu.make_async_copy
    cps = [mk(k_h.at[0, 0:H2], k_ref.at[0:H2], sem.at[0]), mk(v_h.at[0, 0:H2], v_ref.at[0:H2], sem.at[1]),
           mk(h_h.at[:, 0:H2], h_ref.at[:, 0:H2], sem.at[2]),
           mk(k_h.at[0, H2:S], k_ref.at[H2:S], sem.at[3]), mk(v_h.at[0, H2:S], v_ref.at[H2:S], sem.at[4]),
           mk(h_h.at[:, H2:S], h_ref.at[:, H2:S], sem.at[5]),
           mk(wqkv_h, wqkv_ref, sem.at[6]), mk(x_h.at[0], x_ref, sem.at[7]),
           mk(wo_h, wo_ref, sem.at[8]), mk(q_h.at[0], q_ref, sem.at[9])]
    for c in cps: c.start()
    k_s[0:128, :] = jnp.zeros((128, D), I32)
    vT_s[:, 0:256] = jnp.zeros((D // 2, 256), I32)
    ri = lax.broadcasted_iota(I32, (384, 128), 0)
    ci = lax.broadcasted_iota(I32, (384, 128), 1)
    dlt = ci + 256 - ri
    for t in range(3):
        bias_s[t] = jnp.where(((ri < 128) & ((ri <= ci) | (t >= 2))) | ((ri >= 128) & (t >= 1)), 0.0, -1e9)

    mk_s[...] = pk(jnp.where(ri[0:128] > ci[0:128], -1, 0).astype(jnp.int16))
    e8 = (lax.broadcasted_iota(I32, (8, 4), 0) == lax.broadcasted_iota(I32, (8, 4), 1)).astype(BF)
    skT = lax.dot_general(e8, sk_ref[...], NT, preferred_element_type=F32)
    sd = sd_ref[...].astype(F32)
    kf_s[0:8, :] = jnp.zeros((8, D), F32)
    def kvc(j, _):
        r0 = pl.multiple_of(j * 128, 128)
        kf_s[pl.ds(r0 + 8, 128), :] = k_ref[pl.ds(r0, 128), :].astype(F32)
        kk = kf_s[pl.ds(r0, 136), :]
        ks = kk[8:136] * skT[0:1]
        for a in range(1, 4):
            ks = ks + kk[8 - a:136 - a] * skT[a:a + 1]
        kv = ks * v_ref[pl.ds(r0, 128), :].astype(F32)
        kv_s[pl.ds(r0, 128), :] = kv
        F = fw_ref[j % 4]
        U_s[j] = jnp.dot(F, kv.astype(BF), preferred_element_type=F32)
        H_s[j] = lax.dot_general(F, h_ref[:, pl.ds(r0, 128)], NT, preferred_element_type=F32)
    for c in cps[0:3]: c.wait()
    lax.fori_loop(0, 8, kvc, None)
    for c in cps[3:6]: c.wait()
    lax.fori_loop(8, 16, kvc, None)
    for c in cps[6:10]: c.wait()
    wT_s[0:256, :] = pk(wqkv_ref[:, 0:512].T)
    wT_s[256:512, :] = pk(wqkv_ref[:, 1024:1536].T)
    wk_s[...] = pk(wqkv_ref[:, 512:1024])
    wo_s[...] = pk(wo_ref[...])

    def fconv(f0, c0, gate, t):
        ld = lambda R, j, o: R[j, pl.ds(f0 + o, 8), c0:c0 + 128]
        Gr, Gi = [], []
        pr = pi = None
        for m in range(16):
            a, b = ld(H_s, m, 0), ld(H_s, m, 128)
            if gate is not None and m == 0: a = jnp.where(t >= 0, a, gate); b = jnp.where(t >= 0, b, gate)
            Gr.append(a if m == 0 else a + pr); Gi.append(b if m == 0 else b + pi)
            pr, pi = a, b
        for i in range(16):
            yr = yi = None
            for j in range(i + 1):
                ur, ui = ld(U_s, j, 0), ld(U_s, j, 128)
                tr = Gr[i - j] * ur - Gi[i - j] * ui
                ti = Gr[i - j] * ui + Gi[i - j] * ur
                yr = tr if yr is None else yr + tr
                yi = ti if yi is None else yi + ti
            Y_s[i, pl.ds(f0, 8), c0:c0 + 128] = yr
            Y_s[i, pl.ds(f0 + 128, 8), c0:c0 + 128] = yi

    def proj(t, _):
        r0 = pl.multiple_of(t * 256, 256)
        h0 = pl.multiple_of(t * 128, 128)
        xt = x_ref[pl.ds(r0, 256), :]
        qv = lax.dot_general(up(wT_s[...]), xt, NT, preferred_element_type=F32)
        qT_s[:, pl.ds(r0, 256)] = pk((qv[0:512] * qscale).astype(BF))
        vT_s[:, pl.ds(r0 + 256, 256)] = pk(qv[512:1024].astype(BF))
        kk = jnp.dot(xt, up(wk_s[...]), preferred_element_type=F32)
        k_s[pl.ds(h0 + 128, 128), :] = pk(kk.astype(BF))
        for c in range(8):
            gate = None if c < 2 else (qv[160 * (c - 2):160 * (c - 2) + 8, 0:128] if GQ else None)
            fconv(pl.multiple_of(t * 16 + 8 * (c % 2), 8), 128 * (c // 2), gate, t)
    lax.fori_loop(0, 8, proj, None)

    def attn_tile(t, _):
        r0 = pl.multiple_of(t * 128, 128)
        h0 = pl.multiple_of(t * 64, 64)
        tri = lax.broadcasted_iota(I32, (128, 128), 0) > lax.broadcasted_iota(I32, (128, 128), 1)
        tb = jnp.minimum(t, 2)
        mx = {}
        def qk(h):
            g, hh = h // 8, h % 8
            Kg = up(k_s[pl.ds(h0, 192), 128 * g:128 * g + 128])
            q = qT_s[8 * h:8 * h + 8, pl.ds(r0, 128)]
            z = jnp.zeros((8, 128), I32)
            Wm = up(jnp.concatenate([z] * hh + [q] + [z] * (7 - hh), 0))
            s = jnp.dot(Kg, Wm, preferred_element_type=F32)
            s = jnp.concatenate([jnp.where(tri, s[0:128], s[256:384]), s[128:256]], 0) + bias_s[tb, 0:256]
            sc_s[h % 8, 0:256] = s
            mx[h] = jnp.max(s.reshape(32, 8, 128), axis=0)
        def sm(h):
            m = jnp.max(mx[h], axis=0, keepdims=True)
            p = jnp.exp2(sc_s[h % 8, 0:256] - m)
            l = jnp.sum(p, axis=0, keepdims=True)
            pb = pk(p.astype(BF))
            po = pb[0:64] & mk_s[...]
            pp = up(jnp.concatenate([po, pb[64:128], pb[0:64] ^ po], 0))
            vt = up(vT_s[8 * h:8 * h + 8, pl.ds(r0, 384)])
            o = jnp.dot(vt, pp, preferred_element_type=F32)
            oT_s[8 * h:8 * h + 8, :] = pk((o * pl.reciprocal(l, approx=True)).astype(BF))
        for h in range(4): qk(h)
        for qd in range(8):
            for a in range(4):
                if qd < 7: qk(4 * qd + 4 + a)
                sm(4 * qd + a)
        ob = lax.dot_general(up(oT_s[...]), up(wo_s[...]), (((0,), (0,)), ((), ())), preferred_element_type=F32)
        o_ref[pl.ds(r0, 128), 512:1024] = ob.astype(BF)
        j = t
        y = jnp.dot(inv_ref[j % 4], Y_s[j].astype(BF), preferred_element_type=F32)
        y = y + kv_s[pl.ds(r0, 128), :] * sd
        o_ref[pl.ds(r0, 128), 0:512] = (q_ref[pl.ds(r0, 128), :].astype(F32) * y).astype(BF)
        mk(o_ref.at[pl.ds(r0, 128)], o_h.at[0, pl.ds(r0, 128)], osem.at[t]).start()
    lax.fori_loop(0, 16, attn_tile, None)
    for t in range(16):
        mk(o_ref.at[pl.ds(128 * t, 128)], o_h.at[0, pl.ds(128 * t, 128)], osem.at[t]).wait()

@jax.jit
def pallas_concat_heads__ssm_conv_h3__sliding_block__prompt_kernel(A_q, A_k, A_v, A_shift_k, A_ssm_k, A_ssm_D, B_x, B_wqkv, B_wo):
    hb = pl.BlockSpec(memory_space=pl.ANY)
    full = lambda shp: pl.BlockSpec(shp, lambda i: (0,) * len(shp))
    return pl.pallas_call(
        kern, grid=(1,),
        in_specs=[hb, hb, hb, full((D, 4)), hb, full((1, D)), hb, hb, hb, full((4, 256, 128)), full((4, 128, 256))],
        out_specs=hb,
        out_shape=jax.ShapeDtypeStruct((1, S, 2 * D), BF),
        scratch_shapes=[pltpu.VMEM((S, D), BF), pltpu.VMEM((S, D), BF), pltpu.VMEM((S, D), BF), pltpu.VMEM((D, S), BF),
                        pltpu.VMEM((S, D), BF), pltpu.VMEM((D, 3 * D), BF), pltpu.VMEM((D, D), BF), pltpu.VMEM((S, 2 * D), BF),
                        pltpu.SemaphoreType.DMA((10,)), pltpu.SemaphoreType.DMA((16,)),
                        pltpu.VMEM((512, 512), I32), pltpu.VMEM((256, 512), I32), pltpu.VMEM((256, 512), I32),
                        pltpu.VMEM((256, S), I32), pltpu.VMEM((S // 2 + 128, D), I32),
                        pltpu.VMEM((D // 2, S + 256), I32), pltpu.VMEM((256, 128), I32),
                        pltpu.VMEM((3, 384, 128), F32), pltpu.VMEM((8, 384, 128), F32), pltpu.VMEM((64, 128), I32),
                        pltpu.VMEM((S + 8, D), F32), pltpu.VMEM((S, D), F32),
                        pltpu.VMEM((16, 256, D), F32), pltpu.VMEM((16, 256, D), F32), pltpu.VMEM((16, 256, D), F32)],
        compiler_params=pltpu.CompilerParams(vmem_limit_bytes=100 * 2**20),
    )(A_q, A_k, A_v, A_shift_k, A_ssm_k, A_ssm_D.reshape(1, D), B_x, B_wqkv, B_wo, _FW, _INV)
```
